```python
import jax
import jax.numpy as jnp

def _softmax(x, axis=-1):
    return jax.nn.softmax(x, axis=axis)
def _gelu(x):
    return jax.nn.gelu(x, approximate=True)
def _silu(x):
    return jax.nn.silu(x)
def _sigmoid(x):
    return jax.nn.sigmoid(x)
def _layernorm(x, axis=-1, eps=1e-5):
    m = jnp.mean(x, axis=axis, keepdims=True)
    v = jnp.var(x, axis=axis, keepdims=True)
    return (x - m) / jnp.sqrt(v + eps)
def _scatter_add(tgt, idx, src, axis=0):
    return tgt.at[idx].add(src)
def _segment_sum(src, seg, n):
    return jax.ops.segment_sum(src, seg, n)
class _Rng:
    def __init__(self, key):
        self._k = key
    def _next(self):
        self._k, sub = jax.random.split(self._k)
        return sub
    def normal(self, shape):
        return jax.random.normal(self._next(), shape, dtype=jnp.bfloat16)
    def randint(self, lo, hi, shape):
        return jax.random.randint(self._next(), shape, lo, hi, dtype=jnp.int32)
    def uniform(self, shape, lo=0.0, hi=1.0):
        return jax.random.uniform(self._next(), shape, jnp.bfloat16, lo, hi)
    def permutation(self, n):
        return jax.random.permutation(self._next(), n)


kernel_name = 'standalone__instancenorm__prompt'

def setup_inputs():
    _rng = _Rng(jax.random.key(int.from_bytes(__import__("os").urandom(4), "little")))
    _w = (lambda a: (lambda t: t.astype(jnp.bfloat16) if jnp.issubdtype(t.dtype, jnp.floating) else t)(jnp.asarray(a)))
    B, C, H, W = 2, 1024, 2048, 32
    return {
        "x": _w((lambda *s: _rng.normal(s) * 0.05)(B, C, H, W)),
        "g": _w((lambda *s: _rng.normal(s) * 0.05)(C) + 1.0),
        "b": _w((lambda *s: _rng.normal(s) * 0.05)(C)),
    }

def reference(x, g, b):
    mu = x.mean(axis=(-2, -1), keepdims=True)
    var = ((x - mu) * (x - mu)).mean(axis=(-2, -1), keepdims=True)
    xhat = (x - mu) / jnp.sqrt(var + 1e-5)
    return xhat * g.reshape(1, -1, 1, 1) + b.reshape(1, -1, 1, 1)
```

```python
import jax
import jax.numpy as jnp
from jax.experimental import pallas as pl
from jax.experimental.pallas import tpu as pltpu

_EPS = 1e-5
_G = 8
_NP = 4
_WR = 16
_WL = 512
_LC = 512
_K = 4


def _total(a):
    s = jnp.sum(a, axis=0, keepdims=True)
    return jnp.sum(s, axis=1, keepdims=True)


def _normalize(ref, gv, bv):
    w, h = ref.shape
    inv_n = 1.0 / (w * h)
    chunks = [slice(c, c + _LC) for c in range(0, h, _LC)]
    acc = None
    for c in chunks:
        x = ref[:, c].astype(jnp.float32)
        acc = x if acc is None else acc + x
    mu = _total(acc) * inv_n
    acc = None
    for c in chunks:
        d = ref[:, c].astype(jnp.float32) - mu
        acc = d * d if acc is None else acc + d * d
    var = _total(acc) * inv_n
    s = jax.lax.rsqrt(var + _EPS) * gv
    for c in chunks:
        d = ref[:, c].astype(jnp.float32) - mu
        ref[:, c] = (d * s + bv).astype(ref.dtype)


def _kernel(x_hbm, g_ref, b_ref, o_hbm, buf, gs, bs, rsem, wsem):
    n_blk, n_grp, w, h = buf.shape
    per_grp = x_hbm.shape[1] // w
    n_ch = g_ref.shape[0]

    def read(p, j):
        r0 = pl.multiple_of((p * n_blk + j) * w, w)
        return pltpu.make_async_copy(x_hbm.at[:, pl.ds(r0, w), :], buf.at[j], rsem.at[j])

    def write_start(p, j):
        for r in range(0, w, _WR):
            for l in range(0, h, _WL):
                r0 = pl.multiple_of((p * n_blk + j) * w + r, _WR)
                pltpu.make_async_copy(
                    buf.at[j, :, pl.ds(r, _WR), pl.ds(l, _WL)],
                    o_hbm.at[:, pl.ds(r0, _WR), pl.ds(l, _WL)],
                    wsem.at[0]).start()

    def compute(p, j):
        m = p * n_blk + j
        for gi in range(n_grp):
            c = (gi * per_grp) % n_ch + m
            _normalize(buf.at[j, gi], gs[pl.ds(c, 1), :][:, :1], bs[pl.ds(c, 1), :][:, :1])

    pl.loop(0, n_blk)(lambda j: read(0, j).start())
    gs[...] = jnp.broadcast_to(g_ref[...].astype(jnp.float32).reshape(1, n_ch), (128, n_ch)).T
    bs[...] = jnp.broadcast_to(b_ref[...].astype(jnp.float32).reshape(1, n_ch), (128, n_ch)).T

    @pl.loop(0, _NP)
    def _(p):
        @pl.loop(0, n_blk - 1)
        def _(j):
            read(p, j).wait()
            compute(p, j)

        read(p, n_blk - 1).wait()
        pl.loop(0, _K)(lambda j: write_start(p, j))
        compute(p, n_blk - 1)
        pl.loop(_K, n_blk)(lambda j: write_start(p, j))
        pltpu.make_async_copy(buf, buf, wsem.at[0]).wait()

        @pl.when(p + 1 < _NP)
        def _():
            pl.loop(0, n_blk)(lambda j: read(p + 1, j).start())


@jax.jit
def pallas_standalone__instancenorm__prompt_kernel(
    x: jax.Array,
    g: jax.Array,
    b: jax.Array,
):
    B, C, H, W = x.shape
    rows = B * C * W // _G
    xt = x.transpose(0, 1, 3, 2).reshape(_G, rows, H)
    n_blk = rows // W // _NP
    out = pl.pallas_call(
        _kernel,
        in_specs=[
            pl.BlockSpec(memory_space=pl.ANY),
            pl.BlockSpec(memory_space=pltpu.VMEM),
            pl.BlockSpec(memory_space=pltpu.VMEM),
        ],
        out_specs=pl.BlockSpec(memory_space=pl.ANY),
        out_shape=jax.ShapeDtypeStruct(xt.shape, xt.dtype),
        scratch_shapes=[
            pltpu.VMEM((n_blk, _G, W, H), xt.dtype),
            pltpu.VMEM((C, 128), jnp.float32),
            pltpu.VMEM((C, 128), jnp.float32),
            pltpu.SemaphoreType.DMA((n_blk,)),
            pltpu.SemaphoreType.DMA((1,)),
        ],
        compiler_params=pltpu.CompilerParams(vmem_limit_bytes=100 * 1024 * 1024),
    )(xt, g, b)
    return out.reshape(B, C, W, H).transpose(0, 1, 3, 2)
```

```python
import jax
import jax.numpy as jnp
from jax.experimental import pallas as pl
from jax.experimental.pallas import tpu as pltpu

_EPS = 1e-5
_G = 8
_IPG = 8
_NP = 3
_WR = 8
_WL = 1024
_LC = 512
_CG = 4
_K = 2


def _total(a):
    s = jnp.sum(a, axis=0, keepdims=True)
    return jnp.sum(s, axis=1, keepdims=True)


def _normalize(ref, gv, bv):
    w, h = ref.shape
    inv_n = 1.0 / (w * h)
    chunks = [slice(c, c + _LC) for c in range(0, h, _LC)]
    acc = None
    for c in chunks:
        x = ref[:, c].astype(jnp.float32)
        acc = x if acc is None else acc + x
    mu = _total(acc) * inv_n
    acc = None
    for c in chunks:
        d = ref[:, c].astype(jnp.float32) - mu
        acc = d * d if acc is None else acc + d * d
    var = _total(acc) * inv_n
    s = jax.lax.rsqrt(var + _EPS) * gv
    for c in chunks:
        d = ref[:, c].astype(jnp.float32) - mu
        ref[:, c] = (d * s + bv).astype(ref.dtype)


def _kernel(x_hbm, g_ref, b_ref, o_hbm, buf, gs, bs, rsem, wsem):
    n_blk, n_grp, rows, h = x_hbm.shape
    w = rows // _IPG
    n_ch = g_ref.shape[0]
    n_rt = rows // _WR
    n_inst = _CG * _IPG

    def first_block(p):
        return (p * n_blk) // _NP

    def read(a0, a):
        return pltpu.make_async_copy(x_hbm.at[a0 + a], buf.at[a], rsem.at[a])

    def start_reads(a0, n):
        pl.loop(0, n)(lambda a: read(a0, a).start())

    def start_writes(a0, lo, hi):
        @pl.loop(lo * n_rt, hi * n_rt)
        def _(t):
            a = t // n_rt
            r0 = pl.multiple_of((t % n_rt) * _WR, _WR)
            for l in range(0, h, _WL):
                pltpu.make_async_copy(
                    buf.at[a, :, pl.ds(r0, _WR), pl.ds(l, _WL)],
                    o_hbm.at[a0 + a, :, pl.ds(r0, _WR), pl.ds(l, _WL)],
                    wsem.at[a],
                ).start()

    def compute(a0, a):
        @pl.loop(0, n_grp // _CG)
        def _(q):
            c0 = ((a0 + a) * n_grp * _IPG + q * n_inst) % n_ch
            c0 = pl.multiple_of(c0, n_inst)
            gr = gs[pl.ds(c0, n_inst), :]
            br = bs[pl.ds(c0, n_inst), :]
            for i in range(n_inst):
                ref = buf.at[a, q * _CG + i // _IPG, pl.ds((i % _IPG) * w, w)]
                _normalize(ref, gr[i:i + 1, :1], br[i:i + 1, :1])

    start_reads(0, first_block(1))
    gs[...] = jnp.broadcast_to(g_ref[...].astype(jnp.float32).reshape(1, n_ch), (128, n_ch)).T
    bs[...] = jnp.broadcast_to(b_ref[...].astype(jnp.float32).reshape(1, n_ch), (128, n_ch)).T

    @pl.loop(0, _NP)
    def _(p):
        a0, a1 = first_block(p), first_block(p + 1)
        n = a1 - a0

        @pl.loop(0, n - 1)
        def _(a):
            read(a0, a).wait()
            compute(a0, a)

        start_writes(a0, 0, _K)
        read(a0, n - 1).wait()
        compute(a0, n - 1)
        start_writes(a0, _K, n)

        @pl.loop(0, n)
        def _(a):
            pltpu.make_async_copy(buf.at[a], buf.at[a], wsem.at[a]).wait()

        @pl.when(p + 1 < _NP)
        def _():
            start_reads(a1, first_block(p + 2) - a1)


@jax.jit
def pallas_standalone__instancenorm__prompt_kernel(
    x: jax.Array,
    g: jax.Array,
    b: jax.Array,
):
    B, C, H, W = x.shape
    n_blk = B * C // (_G * _IPG)
    assert n_blk * _G * _IPG == B * C and C % (_CG * _IPG) == 0
    max_blk = -(-n_blk // _NP)
    xt = x.transpose(0, 1, 3, 2).reshape(n_blk, _G, _IPG * W, H)
    out = pl.pallas_call(
        _kernel,
        in_specs=[
            pl.BlockSpec(memory_space=pl.ANY),
            pl.BlockSpec(memory_space=pltpu.VMEM),
            pl.BlockSpec(memory_space=pltpu.VMEM),
        ],
        out_specs=pl.BlockSpec(memory_space=pl.ANY),
        out_shape=jax.ShapeDtypeStruct(xt.shape, xt.dtype),
        scratch_shapes=[
            pltpu.VMEM((max_blk,) + xt.shape[1:], xt.dtype),
            pltpu.VMEM((C, 128), jnp.float32),
            pltpu.VMEM((C, 128), jnp.float32),
            pltpu.SemaphoreType.DMA((max_blk,)),
            pltpu.SemaphoreType.DMA((max_blk,)),
        ],
        compiler_params=pltpu.CompilerParams(vmem_limit_bytes=120 * 1024 * 1024),
    )(xt, g, b)
    return out.reshape(B, C, W, H).transpose(0, 1, 3, 2)
```
